```python
import os as _os
_os.environ.setdefault("JAX_PLATFORMS", "cpu")
import jax
import jax.numpy as jnp

def _softmax(x, axis=-1):
    return jax.nn.softmax(x, axis=axis)
def _gelu(x):
    return jax.nn.gelu(x, approximate=True)
def _silu(x):
    return jax.nn.silu(x)
def _sigmoid(x):
    return jax.nn.sigmoid(x)
def _layernorm(x, axis=-1, eps=1e-5):
    m = jnp.mean(x, axis=axis, keepdims=True)
    v = jnp.var(x, axis=axis, keepdims=True)
    return (x - m) / jnp.sqrt(v + eps)
def _scatter_add(tgt, idx, src, axis=0):
    return tgt.at[idx].add(src)
def _segment_sum(src, seg, n):
    return jax.ops.segment_sum(src, seg, n)
class _Rng:
    def __init__(self, key):
        self._k = key
    def _next(self):
        self._k, sub = jax.random.split(self._k)
        return sub
    def normal(self, shape):
        return jax.random.normal(self._next(), shape, dtype=jnp.bfloat16)
    def randint(self, lo, hi, shape):
        return jax.random.randint(self._next(), shape, lo, hi, dtype=jnp.int32)
    def uniform(self, shape, lo=0.0, hi=1.0):
        return jax.random.uniform(self._next(), shape, jnp.bfloat16, lo, hi)
    def permutation(self, n):
        return jax.random.permutation(self._next(), n)


kernel_name = 'sequential_preLN__linear_kernel_hedgehog__dense_activation_squared_relu__prompt'

def setup_inputs():
    _rng = _Rng(jax.random.key(int.from_bytes(__import__("os").urandom(4), "little")))
    _w = (lambda a: (lambda t: t.astype(jnp.bfloat16) if jnp.issubdtype(t.dtype, jnp.floating) else t)(jnp.asarray(a)))
    def _A_setup():
        B, S, D, H = 1, 2048, 512, 32
        Dh = D // H
        return {
            "x": _w((lambda *s: _rng.normal(s) * 0.05)(B, S, D)),
            "wqkv": _w((lambda *s: _rng.normal(s) * 0.2)(D, 3 * D)),
            "w_phi": _w((lambda *s: _rng.normal(s) * 0.2)(H, Dh, Dh) * (Dh ** -0.5)),
            "wo": _w((lambda *s: _rng.normal(s) * 0.05)(D, D)),
        }
    _A_in = _A_setup()

    def _B_setup():
        B, S, D, F = 1, 2048, 512, 1792
        return {
            "x": _w((lambda *s: _rng.normal(s) * 0.05)(B, S, D)),
            "w1": _w((lambda *s: _rng.normal(s) * 0.05)(D, F)),
            "b1": _w((lambda *s: _rng.normal(s) * 0.05)(F)),
            "w2": _w((lambda *s: _rng.normal(s) * 0.05)(F, D)),
            "b2": _w((lambda *s: _rng.normal(s) * 0.05)(D)),
        }
    _B_in = _B_setup()

    return {
        "A_x": _A_in["x"],
        "A_wqkv": _A_in["wqkv"],
        "A_w_phi": _A_in["w_phi"],
        "A_wo": _A_in["wo"],
        "B_x": _B_in["x"],
        "B_w1": _B_in["w1"],
        "B_b1": _B_in["b1"],
        "B_w2": _B_in["w2"],
        "B_b2": _B_in["b2"],
    }

def reference(A_x, A_wqkv, A_w_phi, A_wo, B_x, B_w1, B_b1, B_w2, B_b2):
    def _A_ref(x, wqkv, w_phi, wo):
        B, S, D = x.shape
        H = 32; Dh = D // H
        qkv = (lambda x, *d: x.transpose(*d))((x @ wqkv).reshape(B, S, 3, H, Dh), 2, 0, 3, 1, 4)
        q, k, v = qkv[0], qkv[1], qkv[2]
        pq = jnp.einsum("bhsd,hdf->bhsf", q, w_phi)
        pk = jnp.einsum("bhsd,hdf->bhsf", k, w_phi)
        phi_q = jnp.concatenate([_softmax(pq, axis=-1), _softmax(-pq, axis=-1)], axis=-1)
        phi_k = jnp.concatenate([_softmax(pk, axis=-1), _softmax(-pk, axis=-1)], axis=-1)
        kv = jnp.einsum("bhsf,bhsd->bhfd", phi_k, v)
        z  = jnp.einsum("bhsf->bhf", phi_k)
        num = jnp.einsum("bhqf,bhfd->bhqd", phi_q, kv)
        den = jnp.einsum("bhqf,bhf->bhq", phi_q, z)[..., None] + 1e-6
        o = num / den
        return (lambda x, *d: x.transpose(*d))(o, 0, 2, 1, 3).reshape(B, S, D) @ wo

    def _B_ref(x, w1, b1, w2, b2):
        h = jnp.einsum("bsd,df->bsf", x, w1) + b1
        zero = jnp.zeros_like(h)
        r = jnp.where(h > zero, h, zero)
        h = r * r
        out = jnp.einsum("bsf,fd->bsd", h, w2) + b2
        return out

    x = A_x
    h = x + _A_ref(_layernorm(x, axis=-1), A_wqkv, A_w_phi, A_wo)
    h2 = h + _B_ref(_layernorm(h, axis=-1), B_w1, B_b1, B_w2, B_b2)
    return h2
```

```python
import functools

import jax
import jax.numpy as jnp
from jax import lax
import jax.experimental.pallas as pl
import jax.experimental.pallas.tpu as pltpu

S, D, H, DH, F = 2048, 512, 32, 16, 1792
NC = D // 128
SB = 256
NB = S // SB
KVR = 144

_NT = (((1,), (1,)), ((), ()))
_TN = (((0,), (0,)), ((), ()))
_F32 = jnp.float32
_BF16 = jnp.bfloat16


def _layernorm(x):
    m = jnp.mean(x, axis=-1, keepdims=True)
    xc = x - m
    v = jnp.mean(xc * xc, axis=-1, keepdims=True)
    return xc * lax.rsqrt(v + 1e-5)


def _dual_softmax_t(p):
    n = p.shape[-1]
    p3 = p.reshape(DH, 8, n)
    mx = jnp.max(p3, axis=0, keepdims=True)
    mn = jnp.min(p3, axis=0, keepdims=True)
    ep = jnp.exp(p3 - mx)
    en = jnp.exp(mn - p3)
    rp = 1.0 / jnp.sum(ep, axis=0, keepdims=True)
    rn = 1.0 / jnp.sum(en, axis=0, keepdims=True)
    a = (ep * rp).reshape(128, n).astype(_BF16)
    b = (en * rn).reshape(128, n).astype(_BF16)
    return jnp.concatenate([a, b], axis=0)


def _kernel(x_hbm, wqkv_hbm, wphi_hbm, wo_hbm, w1_hbm, b1_hbm, w2_hbm, b2_hbm,
            out_hbm,
            x_v, wqkv_v, wphi_v, wo_v, w1_v, b1_v, w2_v, b2_v,
            wt_v, wop_v, phiq_v, kv_v, lq_v, out_v,
            wsem, xsem, osem):
    w_copies = [
        pltpu.make_async_copy(wphi_hbm, wphi_v, wsem.at[0]),
        pltpu.make_async_copy(wqkv_hbm, wqkv_v, wsem.at[1]),
        pltpu.make_async_copy(wo_hbm, wo_v, wsem.at[2]),
        pltpu.make_async_copy(w1_hbm, w1_v, wsem.at[3]),
        pltpu.make_async_copy(b1_hbm, b1_v, wsem.at[4]),
        pltpu.make_async_copy(w2_hbm, w2_v, wsem.at[5]),
        pltpu.make_async_copy(b2_hbm, b2_v, wsem.at[6]),
    ]

    def x_copy(i):
        return pltpu.make_async_copy(
            x_hbm.at[pl.ds(i * SB, SB)], x_v.at[pl.ds(i * SB, SB)], xsem.at[i])

    def o_copy(i):
        return pltpu.make_async_copy(
            out_v.at[pl.ds(i * SB, SB)], out_hbm.at[pl.ds(i * SB, SB)], osem.at[i])

    w_copies[0].start()
    w_copies[1].start()
    for i in range(NB):
        x_copy(i).start()
    for cp in w_copies[2:]:
        cp.start()

    row = lax.broadcasted_iota(jnp.int32, (128, 128), 0)
    col = lax.broadcasted_iota(jnp.int32, (128, 128), 1)
    head_mask = (row % 8) == (col // DH)
    perm_t = (col == (row % 8) * DH + row // 8).astype(_BF16)
    er = lax.broadcasted_iota(jnp.int32, (128, DH), 0)
    ec = lax.broadcasted_iota(jnp.int32, (128, DH), 1)
    expand = ((er // 8) == ec).astype(_BF16)

    w_copies[0].wait()
    w_copies[1].wait()
    for c in range(NC):
        a_c = wphi_v[c * 128:(c + 1) * 128, :]
        mx = lax.dot_general(expand, a_c, _NT, preferred_element_type=_F32)
        mt = jnp.where(head_mask, mx, 0.0).astype(_BF16)
        for j, mat in ((0, mt), (1, mt), (2, perm_t)):
            w_c = wqkv_v[:, j * D + c * 128: j * D + (c + 1) * 128]
            wt_v[j * D + c * 128: j * D + (c + 1) * 128, :] = lax.dot_general(
                mat, w_c, _NT, preferred_element_type=_F32).astype(_BF16)
    kv_v[...] = jnp.zeros(kv_v.shape, _F32)

    def phase1(i, carry):
        x_copy(i).wait()
        r0 = pl.multiple_of(i * SB, SB)
        x = x_v[pl.ds(r0, SB), :].astype(_F32)
        xn = _layernorm(x).astype(_BF16)
        qkv_t = lax.dot_general(wt_v[...], xn, _NT,
                                preferred_element_type=_F32)
        ones = jnp.ones((KVR - 128, SB), _BF16)
        for c in range(NC):
            pk = _dual_softmax_t(qkv_t[D + c * 128: D + (c + 1) * 128])
            vt = qkv_t[2 * D + c * 128: 2 * D + (c + 1) * 128].astype(_BF16)
            vt = jnp.concatenate([vt, ones], axis=0)
            kv_v[c] += lax.dot_general(vt, pk, _NT, preferred_element_type=_F32)
            phiq_v[i, c] = _dual_softmax_t(qkv_t[c * 128:(c + 1) * 128])
        return carry

    lax.fori_loop(0, NB, phase1, 0)

    kr = lax.broadcasted_iota(jnp.int32, (KVR, 256), 0)
    kc = lax.broadcasted_iota(jnp.int32, (KVR, 256), 1)
    kmask = (kr % 8) == (kc % 8)
    for c in range(NC):
        lq_v[c] = jnp.where(kmask, kv_v[c], 0.0).astype(_BF16)
    w_copies[2].wait()
    for c in range(NC):
        wop_v[c * 128:(c + 1) * 128, :] = jnp.dot(
            perm_t, wo_v[c * 128:(c + 1) * 128, :],
            preferred_element_type=_F32).astype(_BF16)
    for cp in w_copies[3:]:
        cp.wait()

    def phase2(i, carry):
        r0 = pl.multiple_of(i * SB, SB)
        o_parts = []
        for c in range(NC):
            nd = jnp.dot(lq_v[c], phiq_v[i, c], preferred_element_type=_F32)
            rden = 1.0 / (nd[128:136] + 1e-6)
            o_c = nd[:128].reshape(DH, 8, SB) * rden[None]
            o_parts.append(o_c.reshape(128, SB).astype(_BF16))
        o_t = jnp.concatenate(o_parts, axis=0)
        att = lax.dot_general(o_t, wop_v[...], _TN, preferred_element_type=_F32)
        h = x_v[pl.ds(r0, SB), :].astype(_F32) + att
        hn = _layernorm(h).astype(_BF16)
        h1 = jnp.dot(hn, w1_v[...], preferred_element_type=_F32)
        h1 = h1 + b1_v[...].astype(_F32)
        r = jnp.maximum(h1, 0.0)
        a = (r * r).astype(_BF16)
        y = jnp.dot(a, w2_v[...], preferred_element_type=_F32)
        y = y + b2_v[...].astype(_F32) + h
        out_v[pl.ds(r0, SB), :] = y.astype(_BF16)
        o_copy(i).start()
        return carry

    lax.fori_loop(0, NB, phase2, 0)
    for i in range(NB):
        o_copy(i).wait()


@jax.jit
def pallas_sequential_preLN__linear_kernel_hedgehog__dense_activation_squared_relu__prompt_kernel(
    A_x: jax.Array,
    A_wqkv: jax.Array,
    A_w_phi: jax.Array,
    A_wo: jax.Array,
    B_x: jax.Array,
    B_w1: jax.Array,
    B_b1: jax.Array,
    B_w2: jax.Array,
    B_b2: jax.Array,
):
    del B_x
    x2 = A_x.reshape(S, D)
    wphi2 = A_w_phi.reshape(D, DH)
    b1 = B_b1.reshape(1, F)
    b2 = B_b2.reshape(1, D)
    any_spec = pl.BlockSpec(memory_space=pl.ANY)
    out = pl.pallas_call(
        _kernel,
        in_specs=[any_spec] * 8,
        out_specs=any_spec,
        out_shape=jax.ShapeDtypeStruct((S, D), _BF16),
        scratch_shapes=[
            pltpu.VMEM((S, D), _BF16),
            pltpu.VMEM((D, 3 * D), _BF16),
            pltpu.VMEM((D, DH), _BF16),
            pltpu.VMEM((D, D), _BF16),
            pltpu.VMEM((D, F), _BF16),
            pltpu.VMEM((1, F), _BF16),
            pltpu.VMEM((F, D), _BF16),
            pltpu.VMEM((1, D), _BF16),
            pltpu.VMEM((3 * D, D), _BF16),
            pltpu.VMEM((D, D), _BF16),
            pltpu.VMEM((NB, NC, 256, SB), _BF16),
            pltpu.VMEM((NC, KVR, 256), _F32),
            pltpu.VMEM((NC, KVR, 256), _BF16),
            pltpu.VMEM((S, D), _BF16),
            pltpu.SemaphoreType.DMA((7,)),
            pltpu.SemaphoreType.DMA((NB,)),
            pltpu.SemaphoreType.DMA((NB,)),
        ],
        compiler_params=pltpu.CompilerParams(
            vmem_limit_bytes=100 * 1024 * 1024),
    )(x2, A_wqkv, wphi2, A_wo, B_w1, b1, B_w2, b2)
    return out.reshape(1, S, D)
```

```python
import functools

import jax
import jax.numpy as jnp
from jax import lax
import jax.experimental.pallas as pl
import jax.experimental.pallas.tpu as pltpu

S, D, H, DH, F = 2048, 512, 32, 16, 1792
NC = D // 128
NG = H // 4
SB = 256
NB = S // SB
KVR = 80
OGROUPS = ((0, 4), (4, 7), (7, 8))

_NT = (((1,), (1,)), ((), ()))
_TN = (((0,), (0,)), ((), ()))
_F32 = jnp.float32
_BF16 = jnp.bfloat16
_LOG2E = 1.4426950408889634


def _layernorm(x):
    m = jnp.mean(x, axis=-1, keepdims=True)
    xc = x - m
    v = jnp.mean(xc * xc, axis=-1, keepdims=True)
    return xc * lax.rsqrt(v + 1e-5)


def _dual_softmax_t(p):
    n = p.shape[-1]
    p3 = p.reshape(8, 8, n)
    mx = jnp.max(p3, axis=0)
    mx = jnp.maximum(mx, pltpu.roll(mx, 4, 0))
    mn = jnp.min(p3, axis=0)
    mn = jnp.minimum(mn, pltpu.roll(mn, 4, 0))
    ep = jnp.exp2(p3 - mx[None])
    en = jnp.exp2(mn[None] - p3)
    sp = jnp.sum(ep, axis=0)
    sn = jnp.sum(en, axis=0)
    rp = 1.0 / (sp + pltpu.roll(sp, 4, 0))
    rn = 1.0 / (sn + pltpu.roll(sn, 4, 0))
    a = (ep * rp[None]).reshape(64, n).astype(_BF16)
    b = (en * rn[None]).reshape(64, n).astype(_BF16)
    return jnp.concatenate([a, b], axis=0)


def _kernel(x_hbm, wqkv_hbm, wphi_hbm, wo_hbm, w1_hbm, b1_hbm, w2_hbm, b2_hbm,
            out_hbm,
            x_v, wqkv_v, wphi_v, wo_v, w1_v, b1_v, w2_v, b2_v,
            wt_v, wop_v, phiq_v, out_v,
            wsem, qsem, xsem, osem):
    wphi_cp = pltpu.make_async_copy(wphi_hbm, wphi_v, wsem.at[0])
    late_copies = [
        pltpu.make_async_copy(wo_hbm, wo_v, wsem.at[1]),
        pltpu.make_async_copy(w1_hbm, w1_v, wsem.at[2]),
        pltpu.make_async_copy(b1_hbm, b1_v, wsem.at[3]),
        pltpu.make_async_copy(w2_hbm, w2_v, wsem.at[4]),
        pltpu.make_async_copy(b2_hbm, b2_v, wsem.at[5]),
    ]

    def wq_copy(j):
        return pltpu.make_async_copy(
            wqkv_hbm.at[:, pl.ds(j * D, D)],
            wqkv_v.at[:, pl.ds(j * D, D)], qsem.at[j])

    XG = ((0, 1), (1, 2), (2, 8))

    def x_copy(g):
        a, b = XG[g]
        return pltpu.make_async_copy(
            x_hbm.at[pl.ds(a * SB, (b - a) * SB)],
            x_v.at[pl.ds(a * SB, (b - a) * SB)], xsem.at[g])

    def o_copy(g):
        a, b = OGROUPS[g]
        return pltpu.make_async_copy(
            out_v.at[pl.ds(a * SB, (b - a) * SB)],
            out_hbm.at[pl.ds(a * SB, (b - a) * SB)], osem.at[g])

    wphi_cp.start()
    x_copy(0).start()

    def ln1(i):
        x = x_v[i * SB:(i + 1) * SB, :].astype(_F32)
        return _layernorm(x).astype(_BF16)

    def row_f(r):
        return (r % 64) // 4

    def row_h(r):
        return (r // 64) * 4 + r % 4

    row = lax.broadcasted_iota(jnp.int32, (128, 128), 0)
    col = lax.broadcasted_iota(jnp.int32, (128, 128), 1)
    perm_t = (col == row_h(row) * DH + row_f(row)).astype(_BF16)

    def fold(j, mats):
        for c in range(NC):
            w_c = wqkv_v[:, j * D + c * 128: j * D + (c + 1) * 128]
            wt_v[j * D + c * 128: j * D + (c + 1) * 128, :] = lax.dot_general(
                mats[c], w_c, _NT, preferred_element_type=_F32).astype(_BF16)

    def proj(j, xn):
        return lax.dot_general(wt_v[j * D:(j + 1) * D, :], xn, _NT,
                               preferred_element_type=_F32)

    def q_soft(i, q_t):
        for g in range(NG):
            phiq_v[i, g] = _dual_softmax_t(q_t[g * 64:(g + 1) * 64])

    def k_soft(k_t):
        return [_dual_softmax_t(k_t[g * 64:(g + 1) * 64]) for g in range(NG)]

    ones = jnp.ones((KVR - 64, SB), _BF16)

    def kv_update(kv, pk, v_t):
        new = []
        for g in range(NG):
            vt = v_t[g * 64:(g + 1) * 64].astype(_BF16)
            vt = jnp.concatenate([vt, ones], axis=0)
            u = lax.dot_general(vt, pk[g], _NT, preferred_element_type=_F32)
            new.append(u if kv is None else kv[g] + u)
        return new

    wphi_cp.wait()
    wq_copy(1).start()
    x_copy(0).wait()
    wq_copy(2).start(priority=1)
    xn = ln1(0)
    a = wphi_v[...].reshape(DH * DH, H)
    e3 = (lax.broadcasted_iota(jnp.int32, (H, D), 0)
          == lax.broadcasted_iota(jnp.int32, (H, D), 1) // DH).astype(_BF16)
    r0_ = jnp.dot(a, e3, preferred_element_type=_F32)
    rm = (lax.broadcasted_iota(jnp.int32, (DH * DH, D), 0) // DH
          == lax.broadcasted_iota(jnp.int32, (DH * DH, D), 1) % DH)
    r_ = jnp.where(rm, r0_, 0.0).astype(_BF16)
    lsel = (row_f(lax.broadcasted_iota(jnp.int32, (128, DH * DH), 0))
            == lax.broadcasted_iota(jnp.int32, (128, DH * DH), 1) % DH).astype(_BF16)
    b0 = jnp.dot(lsel, r_, preferred_element_type=_F32)
    hm = (row_h(lax.broadcasted_iota(jnp.int32, (128, D), 0))
          == (lax.broadcasted_iota(jnp.int32, (128, D), 1) // DH) % 8)
    mt_all = jnp.where(hm, b0 * _LOG2E, 0.0).astype(_BF16)
    mts = [mt_all[:, c * 128:(c + 1) * 128] for c in range(NC)]
    wq_copy(1).wait()
    wq_copy(0).start(priority=1)
    x_copy(1).start(priority=1)
    fold(1, mts)
    k_t = proj(1, xn)
    wq_copy(2).wait()
    x_copy(2).start(priority=1)
    pk = k_soft(k_t)
    fold(2, [perm_t] * NC)
    v_t = proj(2, xn)
    kv = kv_update(None, pk, v_t)
    wq_copy(0).wait()
    x_copy(1).wait()
    xn_next = ln1(1)
    fold(0, mts)
    q_soft(0, proj(0, xn))

    for i in range(1, NB):
        xn = xn_next
        pk = k_soft(proj(1, xn))
        if i + 1 < NB:
            q_t = proj(0, xn)
            if i == 1:
                x_copy(2).wait()
                for cp in late_copies:
                    cp.start(priority=1)
            q_soft(i, q_t)
            xn_next = ln1(i + 1)
        v_t = proj(2, xn)
        kv = kv_update(kv, pk, v_t)

    kr = lax.broadcasted_iota(jnp.int32, (KVR, 128), 0)
    kc = lax.broadcasted_iota(jnp.int32, (KVR, 128), 1)
    kmask = (kr % 4) == (kc % 4)
    lq = [jnp.where(kmask, kv[g], 0.0).astype(_BF16) for g in range(NG)]
    for cp in late_copies:
        cp.wait()
    for c in range(NC):
        wop_v[c * 128:(c + 1) * 128, :] = jnp.dot(
            perm_t, wo_v[c * 128:(c + 1) * 128, :],
            preferred_element_type=_F32).astype(_BF16)

    def attn_num(i):
        o_parts = []
        for g in range(NG):
            nd = jnp.dot(lq[g], phiq_v[i, g], preferred_element_type=_F32)
            rden = 1.0 / (nd[64:72] + 1e-6)
            o_g = nd[:64].reshape(8, 8, SB) * rden[None]
            o_parts.append(o_g.reshape(64, SB).astype(_BF16))
        return jnp.concatenate(o_parts, axis=0)

    def attn_wo(i, o_t):
        att = lax.dot_general(o_t, wop_v[...], _TN, preferred_element_type=_F32)
        h = x_v[i * SB:(i + 1) * SB, :].astype(_F32) + att
        return h, _layernorm(h).astype(_BF16)

    def ffn1(hn):
        h1 = jnp.dot(hn, w1_v[...], preferred_element_type=_F32)
        h1 = h1 + b1_v[...].astype(_F32)[None, :]
        r = jnp.maximum(h1, 0.0)
        return (r * r).astype(_BF16)

    def ffn2(i, a, h):
        y = jnp.dot(a, w2_v[...], preferred_element_type=_F32)
        y = y + b2_v[...].astype(_F32)[None, :] + h
        out_v[i * SB:(i + 1) * SB, :] = y.astype(_BF16)

    def last_copy(n):
        r0 = (NB - 1) * SB + n * (SB // 2)
        return pltpu.make_async_copy(
            out_v.at[pl.ds(r0, SB // 2)], out_hbm.at[pl.ds(r0, SB // 2)],
            osem.at[len(OGROUPS) - 1 + n])

    def ffn2_last(a, h):
        hb = SB // 2
        for n in range(2):
            y = jnp.dot(a[n * hb:(n + 1) * hb], w2_v[...],
                        preferred_element_type=_F32)
            y = y + b2_v[...].astype(_F32)[None, :] + h[n * hb:(n + 1) * hb]
            r0 = (NB - 1) * SB + n * hb
            out_v[r0:r0 + hb, :] = y.astype(_BF16)
            last_copy(n).start()

    o_t = attn_num(0)
    q_soft(NB - 1, proj(0, xn))
    h, hn = attn_wo(0, o_t)
    for i in range(NB):
        if i + 1 < NB:
            o_t = attn_num(i + 1)
        a = ffn1(hn)
        if i + 1 < NB:
            nxt = attn_wo(i + 1, o_t)
        if i + 1 < NB:
            ffn2(i, a, h)
            for g, (ga, gb) in enumerate(OGROUPS):
                if gb == i + 1:
                    o_copy(g).start()
        else:
            ffn2_last(a, h)
        if i + 1 < NB:
            h, hn = nxt
    for g in range(len(OGROUPS) - 1):
        o_copy(g).wait()
    last_copy(0).wait()
    last_copy(1).wait()


@jax.jit
def pallas_sequential_preLN__linear_kernel_hedgehog__dense_activation_squared_relu__prompt_kernel(
    A_x: jax.Array,
    A_wqkv: jax.Array,
    A_w_phi: jax.Array,
    A_wo: jax.Array,
    B_x: jax.Array,
    B_w1: jax.Array,
    B_b1: jax.Array,
    B_w2: jax.Array,
    B_b2: jax.Array,
):
    del B_x
    x2 = A_x.reshape(S, D)
    wphi_t = jnp.transpose(A_w_phi, (1, 2, 0))
    any_spec = pl.BlockSpec(memory_space=pl.ANY)
    out = pl.pallas_call(
        _kernel,
        in_specs=[any_spec] * 8,
        out_specs=any_spec,
        out_shape=jax.ShapeDtypeStruct((S, D), _BF16),
        scratch_shapes=[
            pltpu.VMEM((S, D), _BF16),
            pltpu.VMEM((D, 3 * D), _BF16),
            pltpu.VMEM((DH, DH, H), _BF16),
            pltpu.VMEM((D, D), _BF16),
            pltpu.VMEM((D, F), _BF16),
            pltpu.VMEM((F,), _BF16),
            pltpu.VMEM((F, D), _BF16),
            pltpu.VMEM((D,), _BF16),
            pltpu.VMEM((3 * D, D), _BF16),
            pltpu.VMEM((D, D), _BF16),
            pltpu.VMEM((NB, NG, 128, SB), _BF16),
            pltpu.VMEM((S, D), _BF16),
            pltpu.SemaphoreType.DMA((6,)),
            pltpu.SemaphoreType.DMA((3,)),
            pltpu.SemaphoreType.DMA((3,)),
            pltpu.SemaphoreType.DMA((len(OGROUPS) + 1,)),
        ],
        compiler_params=pltpu.CompilerParams(
            vmem_limit_bytes=100 * 1024 * 1024),
    )(x2, A_wqkv, wphi_t, A_wo, B_w1, B_b1, B_w2, B_b2)
    return out.reshape(1, S, D)
```

```python
import jax
import jax.numpy as jnp
from jax import lax
import jax.experimental.pallas as pl
import jax.experimental.pallas.tpu as pltpu

S, D, H, DH, F = 2048, 512, 32, 16, 1792
NC = D // 128
NG = H // 4
SB = 256
NB = S // SB
KVR = 80
XGROUPS = ((0, 1), (1, 2), (2, NB))
OGROUPS = ((0, 4), (4, NB - 1))

_NT = (((1,), (1,)), ((), ()))
_TN = (((0,), (0,)), ((), ()))
_F32 = jnp.float32
_BF16 = jnp.bfloat16
_LOG2E = 1.4426950408889634


def _layernorm(x):
    m = jnp.mean(x, axis=-1, keepdims=True)
    xc = x - m
    v = jnp.mean(xc * xc, axis=-1, keepdims=True)
    return xc * lax.rsqrt(v + 1e-5)


def _dual_softmax_t(p):
    n = p.shape[-1]
    p3 = p.reshape(8, 8, n)
    mx = jnp.max(p3, axis=0)
    mx = jnp.maximum(mx, pltpu.roll(mx, 4, 0))
    mn = jnp.min(p3, axis=0)
    mn = jnp.minimum(mn, pltpu.roll(mn, 4, 0))
    ep = jnp.exp2(p3 - mx[None])
    en = jnp.exp2(mn[None] - p3)
    sp = jnp.sum(ep, axis=0)
    sn = jnp.sum(en, axis=0)
    rp = 1.0 / (sp + pltpu.roll(sp, 4, 0))
    rn = 1.0 / (sn + pltpu.roll(sn, 4, 0))
    a = (ep * rp[None]).reshape(64, n).astype(_BF16)
    b = (en * rn[None]).reshape(64, n).astype(_BF16)
    return jnp.concatenate([a, b], axis=0)


def _kernel(x_hbm, wqkv_hbm, wphi_hbm, wo_hbm, w1_hbm, b1_hbm, w2_hbm, b2_hbm,
            out_hbm,
            x_v, wqkv_v, wphi_v, wo_v, w1_v, b1_v, w2_v, b2_v,
            wt_v, wop_v, phiq_v, out_v,
            wsem, qsem, xsem, osem):
    wphi_cp = pltpu.make_async_copy(wphi_hbm, wphi_v, wsem.at[0])
    late_copies = [
        pltpu.make_async_copy(wo_hbm, wo_v, wsem.at[1]),
        pltpu.make_async_copy(w1_hbm, w1_v, wsem.at[2]),
        pltpu.make_async_copy(b1_hbm, b1_v, wsem.at[3]),
        pltpu.make_async_copy(w2_hbm, w2_v, wsem.at[4]),
        pltpu.make_async_copy(b2_hbm, b2_v, wsem.at[5]),
    ]

    def w_copy(j):
        return pltpu.make_async_copy(
            wqkv_hbm.at[:, pl.ds(j * D, D)], wqkv_v.at[j], qsem.at[j])

    def x_copy(g):
        a, b = XGROUPS[g]
        return pltpu.make_async_copy(
            x_hbm.at[pl.ds(a * SB, (b - a) * SB)],
            x_v.at[pl.ds(a * SB, (b - a) * SB)], xsem.at[g])

    def o_copy(g):
        a, b = OGROUPS[g]
        return pltpu.make_async_copy(
            out_v.at[pl.ds(a * SB, (b - a) * SB)],
            out_hbm.at[pl.ds(a * SB, (b - a) * SB)], osem.at[g])

    def o_last_copy(n):
        r0 = (NB - 1) * SB + n * (SB // 2)
        return pltpu.make_async_copy(
            out_v.at[pl.ds(r0, SB // 2)], out_hbm.at[pl.ds(r0, SB // 2)],
            osem.at[len(OGROUPS) + n])

    wphi_cp.start()
    x_copy(0).start()

    def row_f(r):
        return (r % 64) // 4

    def row_h(r):
        return (r // 64) * 4 + r % 4

    row = lax.broadcasted_iota(jnp.int32, (128, 128), 0)
    col = lax.broadcasted_iota(jnp.int32, (128, 128), 1)
    perm_t = (col == row_h(row) * DH + row_f(row)).astype(_BF16)

    def ln1(i):
        x = x_v[i * SB:(i + 1) * SB, :].astype(_F32)
        return _layernorm(x).astype(_BF16)

    def fold(j, mats):
        for c in range(NC):
            w_c = wqkv_v[j, :, c * 128:(c + 1) * 128]
            wt = lax.dot_general(mats[c], w_c, _NT, preferred_element_type=_F32)
            if j != 2:
                wt = wt * _LOG2E
            wt_v[j * D + c * 128: j * D + (c + 1) * 128, :] = wt.astype(_BF16)

    def proj(j, xn):
        return lax.dot_general(wt_v[j * D:(j + 1) * D, :], xn, _NT,
                               preferred_element_type=_F32)

    def q_soft(i, q_t):
        for g in range(NG):
            phiq_v[i, g] = _dual_softmax_t(q_t[g * 64:(g + 1) * 64])

    def k_soft(k_t):
        return [_dual_softmax_t(k_t[g * 64:(g + 1) * 64]) for g in range(NG)]

    ones = jnp.ones((KVR - 64, SB), _BF16)

    def kv_update(kv, pk, v_t):
        new = []
        for g in range(NG):
            vt = v_t[g * 64:(g + 1) * 64].astype(_BF16)
            vt = jnp.concatenate([vt, ones], axis=0)
            u = lax.dot_general(vt, pk[g], _NT, preferred_element_type=_F32)
            new.append(u if kv is None else kv[g] + u)
        return new

    wphi_cp.wait()
    w_copy(1).start()
    x_copy(0).wait()
    w_copy(2).start(priority=1)
    xn = ln1(0)
    a = wphi_v[...].reshape(DH * DH, H)
    e3 = (lax.broadcasted_iota(jnp.int32, (H, D), 0)
          == lax.broadcasted_iota(jnp.int32, (H, D), 1) // DH).astype(_BF16)
    r0_ = jnp.dot(a, e3, preferred_element_type=_F32)
    rm = (lax.broadcasted_iota(jnp.int32, (DH * DH, D), 0) // DH
          == lax.broadcasted_iota(jnp.int32, (DH * DH, D), 1) % DH)
    r_ = jnp.where(rm, r0_, 0.0).astype(_BF16)
    lsel = (row_f(lax.broadcasted_iota(jnp.int32, (128, DH * DH), 0))
            == lax.broadcasted_iota(jnp.int32, (128, DH * DH), 1) % DH
            ).astype(_BF16)
    b0 = jnp.dot(lsel, r_, preferred_element_type=_F32)
    hm = (row_h(lax.broadcasted_iota(jnp.int32, (128, D), 0))
          == (lax.broadcasted_iota(jnp.int32, (128, D), 1) // DH) % 8)
    mt_all = jnp.where(hm, b0, 0.0).astype(_BF16)
    mts = [mt_all[:, c * 128:(c + 1) * 128] for c in range(NC)]

    w_copy(1).wait()
    w_copy(0).start(priority=1)
    x_copy(1).start(priority=1)
    fold(1, mts)
    k_t = proj(1, xn)
    w_copy(2).wait()
    x_copy(2).start(priority=1)
    pk = k_soft(k_t)
    fold(2, [perm_t] * NC)
    v_t = proj(2, xn)
    kv = kv_update(None, pk, v_t)
    w_copy(0).wait()
    x_copy(1).wait()
    xn_next = ln1(1)
    fold(0, mts)
    q_soft(0, proj(0, xn))

    for i in range(1, NB):
        xn = xn_next
        pk = k_soft(proj(1, xn))
        if i + 1 < NB:
            q_t = proj(0, xn)
            if i == 1:
                x_copy(2).wait()
                for cp in late_copies:
                    cp.start(priority=1)
            q_soft(i, q_t)
            xn_next = ln1(i + 1)
        v_t = proj(2, xn)
        kv = kv_update(kv, pk, v_t)

    kr = lax.broadcasted_iota(jnp.int32, (KVR, 128), 0)
    kc = lax.broadcasted_iota(jnp.int32, (KVR, 128), 1)
    kmask = (kr % 4) == (kc % 4)
    lq = [jnp.where(kmask, kv[g], 0.0).astype(_BF16) for g in range(NG)]
    for cp in late_copies:
        cp.wait()
    for c in range(NC):
        wop_v[c * 128:(c + 1) * 128, :] = jnp.dot(
            perm_t, wo_v[c * 128:(c + 1) * 128, :],
            preferred_element_type=_F32).astype(_BF16)

    def attn_num(i):
        o_parts = []
        for g in range(NG):
            nd = jnp.dot(lq[g], phiq_v[i, g], preferred_element_type=_F32)
            rden = 1.0 / (nd[64:72] + 1e-6)
            o_g = nd[:64].reshape(8, 8, SB) * rden[None]
            o_parts.append(o_g.reshape(64, SB).astype(_BF16))
        return jnp.concatenate(o_parts, axis=0)

    def attn_wo(i, o_t):
        att = lax.dot_general(o_t, wop_v[...], _TN, preferred_element_type=_F32)
        h = x_v[i * SB:(i + 1) * SB, :].astype(_F32) + att
        return h, _layernorm(h).astype(_BF16)

    def ffn1(hn):
        h1 = jnp.dot(hn, w1_v[...], preferred_element_type=_F32)
        h1 = h1 + b1_v[...].astype(_F32)[None, :]
        r = jnp.maximum(h1, 0.0)
        return (r * r).astype(_BF16)

    def ffn2(r0, act, h):
        y = jnp.dot(act, w2_v[...], preferred_element_type=_F32)
        y = y + b2_v[...].astype(_F32)[None, :] + h
        out_v[r0:r0 + act.shape[0], :] = y.astype(_BF16)

    o_t = attn_num(0)
    q_soft(NB - 1, proj(0, xn))
    h, hn = attn_wo(0, o_t)
    for i in range(NB - 1):
        o_t = attn_num(i + 1)
        act = ffn1(hn)
        nxt = attn_wo(i + 1, o_t)
        ffn2(i * SB, act, h)
        for g, (_, gb) in enumerate(OGROUPS):
            if gb == i + 1:
                o_copy(g).start()
        h, hn = nxt
    act = ffn1(hn)
    hb = SB // 2
    for n in range(2):
        ffn2((NB - 1) * SB + n * hb, act[n * hb:(n + 1) * hb],
             h[n * hb:(n + 1) * hb])
        o_last_copy(n).start()
    for g in range(len(OGROUPS)):
        o_copy(g).wait()
    o_last_copy(0).wait()
    o_last_copy(1).wait()


@jax.jit
def pallas_sequential_preLN__linear_kernel_hedgehog__dense_activation_squared_relu__prompt_kernel(
    A_x: jax.Array,
    A_wqkv: jax.Array,
    A_w_phi: jax.Array,
    A_wo: jax.Array,
    B_x: jax.Array,
    B_w1: jax.Array,
    B_b1: jax.Array,
    B_w2: jax.Array,
    B_b2: jax.Array,
):
    del B_x
    x2 = A_x.reshape(S, D)
    wphi_t = jnp.transpose(A_w_phi, (1, 2, 0))
    any_spec = pl.BlockSpec(memory_space=pl.ANY)
    out = pl.pallas_call(
        _kernel,
        in_specs=[any_spec] * 8,
        out_specs=any_spec,
        out_shape=jax.ShapeDtypeStruct((S, D), _BF16),
        scratch_shapes=[
            pltpu.VMEM((S, D), _BF16),
            pltpu.VMEM((3, D, D), _BF16),
            pltpu.VMEM((DH, DH, H), _BF16),
            pltpu.VMEM((D, D), _BF16),
            pltpu.VMEM((D, F), _BF16),
            pltpu.VMEM((F,), _BF16),
            pltpu.VMEM((F, D), _BF16),
            pltpu.VMEM((D,), _BF16),
            pltpu.VMEM((3 * D, D), _BF16),
            pltpu.VMEM((D, D), _BF16),
            pltpu.VMEM((NB, NG, 128, SB), _BF16),
            pltpu.VMEM((S, D), _BF16),
            pltpu.SemaphoreType.DMA((6,)),
            pltpu.SemaphoreType.DMA((3,)),
            pltpu.SemaphoreType.DMA((len(XGROUPS),)),
            pltpu.SemaphoreType.DMA((len(OGROUPS) + 2,)),
        ],
        compiler_params=pltpu.CompilerParams(
            vmem_limit_bytes=100 * 1024 * 1024),
    )(x2, A_wqkv, wphi_t, A_wo, B_w1, B_b1, B_w2, B_b2)
    return out.reshape(1, S, D)
```
